```python
import os as _os
_os.environ.setdefault("JAX_PLATFORMS", "cpu")
import jax
import jax.numpy as jnp

def _softmax(x, axis=-1):
    return jax.nn.softmax(x, axis=axis)
def _gelu(x):
    return jax.nn.gelu(x, approximate=True)
def _silu(x):
    return jax.nn.silu(x)
def _sigmoid(x):
    return jax.nn.sigmoid(x)
def _layernorm(x, axis=-1, eps=1e-5):
    m = jnp.mean(x, axis=axis, keepdims=True)
    v = jnp.var(x, axis=axis, keepdims=True)
    return (x - m) / jnp.sqrt(v + eps)
def _scatter_add(tgt, idx, src, axis=0):
    return tgt.at[idx].add(src)
def _segment_sum(src, seg, n):
    return jax.ops.segment_sum(src, seg, n)
class _Rng:
    def __init__(self, key):
        self._k = key
    def _next(self):
        self._k, sub = jax.random.split(self._k)
        return sub
    def normal(self, shape):
        return jax.random.normal(self._next(), shape, dtype=jnp.bfloat16)
    def randint(self, lo, hi, shape):
        return jax.random.randint(self._next(), shape, lo, hi, dtype=jnp.int32)
    def uniform(self, shape, lo=0.0, hi=1.0):
        return jax.random.uniform(self._next(), shape, jnp.bfloat16, lo, hi)
    def permutation(self, n):
        return jax.random.permutation(self._next(), n)


kernel_name = 'recurrent_scan__ssm_conv_s4__mixer_s_mlp__prompt'

def setup_inputs():
    _rng = _Rng(jax.random.key(int.from_bytes(__import__("os").urandom(4), "little")))
    _w = (lambda a: (lambda t: t.astype(jnp.bfloat16) if jnp.issubdtype(t.dtype, jnp.floating) else t)(jnp.asarray(a)))
    def _A_setup():
        B, L, D, N = 1, 2048, 512, 128
        A_re = -jnp.exp((lambda *s: _rng.normal(s) * 0.1)(D, N))
        A_im = jnp.pi * (lambda *s: _rng.normal(s) * 0.1)(D, N)
        B_re = (lambda *s: _rng.normal(s) * 0.1)(D, N)
        B_im = (lambda *s: _rng.normal(s) * 0.1)(D, N)
        C_re = (lambda *s: _rng.normal(s) * 0.1)(D, N)
        C_im = (lambda *s: _rng.normal(s) * 0.1)(D, N)
        log_dt = (lambda *s: _rng.normal(s) * 0.1)(D) * 0.5 - 4.0
        Dskip = (lambda *s: _rng.normal(s) * 0.05)(D)
        return {
            "u": _w((lambda *s: _rng.normal(s) * 0.05)(B, L, D)),
            "A_re": _w(A_re),
            "A_im": _w(A_im),
            "B_re": _w(B_re),
            "B_im": _w(B_im),
            "C_re": _w(C_re),
            "C_im": _w(C_im),
            "log_dt": _w(log_dt),
            "Dskip": _w(Dskip),
        }
    _A_in = _A_setup()

    def _B_setup():
        B, S, D, F = 1, 2048, 512, 1376
        return {
            "x":  _w((lambda *s: _rng.normal(s) * 0.05)(B, S, D)),
            "w1": _w((lambda *s: _rng.normal(s) * 0.8)(D, D) * (D ** -0.5)),
            "w2": _w((lambda *s: _rng.normal(s) * 0.8)(D, D) * (D ** -0.5)),
            "w3": _w((lambda *s: _rng.normal(s) * 0.8)(D, F) * (D ** -0.5)),
            "w4": _w((lambda *s: _rng.normal(s) * 0.8)(F, D) * (F ** -0.5)),
        }
    _B_in = _B_setup()

    return {
        "A_u": _A_in["u"],
        "A_A_re": _A_in["A_re"],
        "A_A_im": _A_in["A_im"],
        "A_B_re": _A_in["B_re"],
        "A_B_im": _A_in["B_im"],
        "A_C_re": _A_in["C_re"],
        "A_C_im": _A_in["C_im"],
        "A_log_dt": _A_in["log_dt"],
        "A_Dskip": _A_in["Dskip"],
        "B_x": _B_in["x"],
        "B_w1": _B_in["w1"],
        "B_w2": _B_in["w2"],
        "B_w3": _B_in["w3"],
        "B_w4": _B_in["w4"],
    }

def reference(A_u, A_A_re, A_A_im, A_B_re, A_B_im, A_C_re, A_C_im, A_log_dt, A_Dskip, B_x, B_w1, B_w2, B_w3, B_w4):
    def _A_ref(u, A_re, A_im, B_re, B_im, C_re, C_im, log_dt, Dskip):
        Bsz, L, D = u.shape
        dt = jnp.exp(log_dt)[:, None]
        A = A_re + 1j * A_im
        Bc = B_re + 1j * B_im
        Cc = C_re + 1j * C_im
        logdA = dt * A
        dB = dt * Bc
        l = (lambda x, dt: x.astype(dt))(jnp.arange(L), A_re.dtype)
        P = jnp.exp(logdA[:, :, None] * l[None, None, :])
        K = jnp.einsum("dn,dnl,dn->dl", Cc, P, dB).real
        L2 = 2 * L
        Kp = jnp.pad(K, ((0, 0), (0, L)))
        up = (lambda x, *d: x.transpose(*d))(u, 0, 2, 1)
        up = jnp.pad(up, ((0, 0), (0, 0), (0, L)))
        Kf = (lambda x, axes=(-2,-1): jnp.fft.rfft2(x.astype(jnp.float32), axes=axes))(Kp[:, None, :], axes=(-2, -1))
        Uf = (lambda x, axes=(-2,-1): jnp.fft.rfft2(x.astype(jnp.float32), axes=axes))(up[:, :, None, :], axes=(-2, -1))
        Yf = Uf * Kf[None, :, :, :]
        y = (lambda x, s, axes=(-2,-1): jnp.fft.irfft2(x, s=s, axes=axes).astype(jnp.bfloat16))(Yf, (1, L2), axes=(-2, -1))[:, :, 0, :L]
        y = (lambda x, *d: x.transpose(*d))(y, 0, 2, 1) + u * Dskip[None, None, :]
        return y

    def _B_ref(x, w1, w2, w3, w4):
        B, S, D = x.shape
        h = _gelu(_layernorm(x, axis=-1) @ w1)
        c = D // 4
        g0 = jnp.pad(h[:, :, 0*c:1*c], ((0, 0), (1, 0), (0, 0)))[:, :S, :]
        g1 = jnp.pad(h[:, :, 1*c:2*c], ((0, 0), (0, 1), (0, 0)))[:, 1:, :]
        g2 = jnp.pad(h[:, :, 2*c:3*c], ((0, 0), (2, 0), (0, 0)))[:, :S, :]
        g3 = jnp.pad(h[:, :, 3*c:   ], ((0, 0), (0, 2), (0, 0)))[:, 2:, :]
        hs = jnp.concatenate([g0, g1, g2, g3], axis=-1) @ w2
        x1 = x + hs
        h2 = _gelu(_layernorm(x1, axis=-1) @ w3) @ w4
        return x1 + h2

    x = A_u
    xn = _layernorm(x, axis=-1)
    s = _A_ref(xn, A_A_re, A_A_im, A_B_re, A_B_im, A_C_re, A_C_im, A_log_dt, A_Dskip)
    g = _silu(_B_ref(xn, B_w1, B_w2, B_w3, B_w4))
    return x + s * g
```

```python
import functools
import numpy as np
import jax
import jax.numpy as jnp
import jax.experimental.pallas as pl
import jax.experimental.pallas.tpu as pltpu

L = 2048
D = 512
N = 128
FF = 1376
BLK = 256
NB = L // BLK
HALO = 16
CH = 8
FFP = 1376
FC = 256
PINS = {0: 32}
S4 = (0, 3, 6)

_EXPS = list(range(32)) + list(range(32, 64, 2)) + list(range(64, 128, 4))
_ROWV = ([32 * j for j in range(8)] + [256 + 64 * j for j in range(4)]
         + [512 + 128 * j for j in range(4)] + [1024 + 128 * j for j in range(8)] + [2048])


def _bf16_round_int(l):
    if l < 256:
        return l
    s = 1 << (l.bit_length() - 8)
    q, r = divmod(l, s)
    if 2 * r > s or (2 * r == s and q % 2 == 1):
        q += 1
    return q * s


@functools.lru_cache(maxsize=None)
def _tables():
    om = np.concatenate([np.arange(0, BLK, 2), np.arange(1, BLK, 2)]).astype(np.float64)
    th = 2.0 * np.pi * (om + 0.5) / (2 * BLK)
    j = np.arange(BLK, dtype=np.float64)
    f = np.concatenate([np.cos(th[:, None] * j[None, :]), -np.sin(th[:, None] * j[None, :])], 0)
    m = BLK + j
    g = np.concatenate([np.cos(th[None, :] * m[:, None]), -np.sin(th[None, :] * m[:, None])], 1) / BLK
    pairs = [(0, 0, 1, 32), (0, 2, 3, 32), (1, 4, -1, 0), (1, 5, -1, 0)] + [
        (q, q + 4, q + 5, 1) for q in range(2, NB)]
    own_rows = {0: range(0, 8), 1: range(8, 12)}
    own_rows.update({q: (2 * q + 8, 2 * q + 9) for q in range(2, NB)})
    fk_all = np.zeros((len(pairs), 2 * BLK, 128))
    for l in range(L):
        q = l // BLK
        v = _bf16_round_int(l)
        if q >= 2 and v == (q + 1) * BLK:
            assert _ROWV[2 * q + 10] == v
            idx, lane = q + 2, 1
        else:
            r = max(rr for rr in own_rows[q] if _ROWV[rr] <= v)
            lane = (r % 2) * 64 + _EXPS.index(v - _ROWV[r])
            if q == 0:
                assert lane % 64 < 32
                idx, lane = r // 4, lane + 32 * ((r // 2) % 2)
            elif q == 1:
                idx = r // 2 - 2
            else:
                assert lane != 1
                idx = q + 2
        fk_all[idx, :, lane] += f[:, l - q * BLK]
    return (f.astype(np.float32), g.astype(np.float32), fk_all.astype(np.float32), tuple(pairs))


def _cmul(a, b):
    return a[0] * b[0] - a[1] * b[1], a[0] * b[1] + a[1] * b[0]


def _layernorm(x):
    m = jnp.mean(x, axis=-1, keepdims=True)
    xc = x - m
    v = jnp.mean(xc * xc, axis=-1, keepdims=True)
    return xc * jax.lax.rsqrt(v + 1e-5)


def _kernel(pairs,
            x_hbm, are_hbm, aim_hbm, bre_hbm, bim_hbm, cre_hbm, cim_hbm, ldt_hbm, dsk_hbm,
            w1_hbm, w2_hbm, w3_hbm, w4_hbm, f_hbm, g_hbm, fk_hbm,
            o_ref,
            xs, w1, w2, w3, w4, f_ref, g_ref, fk_ref, sems,
            are_ref, aim_ref, bre_ref, bim_ref, cre_ref, cim_ref, ldt_ref, dsk_ref, psems,
            lam_r, lam_i, c_r, c_i, vbuf, ubuf, vbuf2, ubuf2, ps, kf, ksv, zs, hbuf):
    i = pl.program_id(0)
    bf = jnp.bfloat16
    f32 = jnp.float32

    def copies():
        return (pltpu.make_async_copy(x_hbm, xs.at[pl.ds(HALO, L)], sems.at[0]),
                pltpu.make_async_copy(w1_hbm, w1, sems.at[1]),
                pltpu.make_async_copy(w2_hbm, w2, sems.at[2]),
                pltpu.make_async_copy(w3_hbm, w3, sems.at[3]),
                pltpu.make_async_copy(w4_hbm, w4, sems.at[4]),
                pltpu.make_async_copy(f_hbm, f_ref, sems.at[5]),
                pltpu.make_async_copy(g_hbm, g_ref, sems.at[6]),
                pltpu.make_async_copy(dsk_hbm, dsk_ref, psems.at[7]))

    def front(blk):
        r0 = pl.multiple_of(jnp.minimum(blk, NB - 1) * BLK, BLK)
        xe = xs[pl.ds(r0, BLK + 2 * HALO), :].astype(f32)
        xn_e = _layernorm(xe).astype(bf)
        xn = xn_e[HALO:HALO + BLK]
        xf = jnp.dot(f_ref[...], xn, preferred_element_type=f32)
        zs[1 + blk, 0:2 * BLK] = xf
        zs[1 + blk, 2 * BLK:3 * BLK] = xf[0:BLK] + xf[BLK:2 * BLK]
        hn = _layernorm(xn_e.astype(f32)).astype(bf)
        h = jax.nn.gelu(jnp.dot(hn, w1[...], preferred_element_type=f32), approximate=True)
        grow = r0 - HALO + jax.lax.broadcasted_iota(jnp.int32, (BLK + 2 * HALO, 1), 0)
        h = jnp.where((grow >= 0) & (grow < L), h, 0.0)
        c4 = D // 4
        hs_in = jnp.concatenate([
            h[HALO - 1:HALO - 1 + BLK, 0:c4],
            h[HALO + 1:HALO + 1 + BLK, c4:2 * c4],
            h[HALO - 2:HALO - 2 + BLK, 2 * c4:3 * c4],
            h[HALO + 2:HALO + 2 + BLK, 3 * c4:4 * c4]], axis=1).astype(bf)
        x1 = xn.astype(f32) + jnp.dot(hs_in, w2[...], preferred_element_type=f32)
        return _layernorm(x1).astype(bf), x1, xn

    @pl.when(i == 0)
    def _prologue():
        a_copies = (pltpu.make_async_copy(ldt_hbm, ldt_ref, psems.at[0]),
                    pltpu.make_async_copy(are_hbm, are_ref, psems.at[1]),
                    pltpu.make_async_copy(aim_hbm, aim_ref, psems.at[2]))
        bc_copies = (pltpu.make_async_copy(bre_hbm, bre_ref, psems.at[3]),
                     pltpu.make_async_copy(bim_hbm, bim_ref, psems.at[4]),
                     pltpu.make_async_copy(cre_hbm, cre_ref, psems.at[5]),
                     pltpu.make_async_copy(cim_hbm, cim_ref, psems.at[6]))
        for c in a_copies + bc_copies:
            c.start()
        xs[pl.ds(0, HALO), :] = jnp.zeros((HALO, D), bf)
        xs[pl.ds(HALO + L, HALO), :] = jnp.zeros((HALO, D), bf)
        zs[0] = jnp.zeros((3 * BLK, D), f32)
        for c in a_copies:
            c.wait()
        dt_row = jnp.exp(ldt_ref[...].astype(f32).reshape(1, D)).astype(bf).astype(f32)
        dt = jnp.broadcast_to(dt_row, (N, D)).T
        mag = jnp.exp(dt * are_ref[...].astype(f32))
        ang = dt * aim_ref[...].astype(f32)
        lam_r[...] = mag * jnp.cos(ang)
        lam_i[...] = mag * jnp.sin(ang)
        for c in bc_copies:
            c.wait()
        fk_copy = pltpu.make_async_copy(fk_hbm, fk_ref, sems.at[7])
        fk_copy.start()
        for c in copies():
            c.start()
        br = dt * bre_ref[...].astype(f32)
        bi = dt * bim_ref[...].astype(f32)
        cr = cre_ref[...].astype(f32)
        ci = cim_ref[...].astype(f32)
        c_r[...] = cr * br - ci * bi
        c_i[...] = cr * bi + ci * br

        lane = jax.lax.broadcasted_iota(jnp.int32, (16, 128), 1)
        low = lane < 64

        def gen(c, vb, ub):
            rows = pl.ds(pl.multiple_of(c * CH, CH), CH)
            def put_v(ex):
                e = _EXPS.index(ex)
                vb[pl.ds(e * CH, CH), :] = pw[ex][0]
                vb[pl.ds((64 + e) * CH, CH), :] = pw[ex][1]

            pw = {1: (lam_r[rows, :], lam_i[rows, :])}
            put_v(1)
            yield
            for k in range(2, 32):
                h = 1 << (k.bit_length() - 1)
                pw[k] = _cmul(pw[h // 2], pw[h // 2]) if k == h else _cmul(pw[h], pw[k - h])
                put_v(k)
                if k in (12, 22):
                    yield
            pw[32] = _cmul(pw[16], pw[16])
            pw[64] = _cmul(pw[32], pw[32])
            pw[96] = _cmul(pw[64], pw[32])
            put_v(32)
            put_v(64)
            put_v(96)
            yield
            pw[128] = _cmul(pw[64], pw[64])
            for k in range(34, 64, 2):
                pw[k] = _cmul(pw[32], pw[k - 32])
                put_v(k)
            yield
            for k in range(68, 96, 4):
                pw[k] = _cmul(pw[64], pw[k - 64])
                put_v(k)
            for k in range(100, 128, 4):
                pw[k] = _cmul(pw[96], pw[k - 96])
                put_v(k)
            yield
            for k, (k1, k2) in ((160, (128, 32)), (192, (128, 64)), (224, (128, 96)), (256, (128, 128)),
                                (384, (256, 128)), (512, (256, 256)), (640, (512, 128)),
                                (768, (512, 256)), (896, (512, 384)), (1024, (512, 512))):
                pw[k] = _cmul(pw[k1], pw[k2])
            cb = {0: (c_r[rows, :], c_i[rows, :])}
            for base in (256, 512, 1024):
                cb[base] = _cmul(cb[0], pw[base])
            yield
            for r, v1 in enumerate(_ROWV):
                base = max(bb for bb in cb if bb <= v1)
                u = cb[base] if v1 == base else _cmul(cb[base], pw[v1 - base])
                pos = (r % 2) * 16 + r // 2
                ub[pl.ds(pos * CH, CH), :] = u[0]
                ub[pl.ds((32 + pos) * CH, CH), :] = u[1]
                if r == 12:
                    yield

        def mm(c, vb, ub):
            for j in range(CH):
                vt = vb[pl.ds(j, 128, stride=CH), :].astype(bf)
                ut = ub[pl.ds(j, 64, stride=CH), :].astype(bf)
                out = jax.lax.dot_general(ut, vt, (((1,), (1,)), ((), ())),
                                          preferred_element_type=f32)
                pk = jnp.where(low, out[0:16] - pltpu.roll(out[32:48], 64, 1),
                               pltpu.roll(out[16:32], 64, 1) - out[48:64])
                ps[pl.ds(pl.multiple_of((c * CH + j) * 16, 16), 16), :] = pk
                yield

        def interleave(g1, g2):
            done1 = done2 = False
            while not (done1 and done2):
                if not done1:
                    done1 = next(g1, 'end') == 'end'
                if not done2:
                    done2 = next(g2, 'end') == 'end'

        for vb, ub in ((vbuf, ubuf), (vbuf2, ubuf2)):
            ub[...] = jnp.zeros(ub.shape, f32)
            vb[pl.ds(0, CH), :] = jnp.ones((CH, N), f32)
            vb[pl.ds(64 * CH, CH), :] = jnp.zeros((CH, N), f32)
        NCH = D // CH
        for _ in gen(0, vbuf, ubuf):
            pass

        def two(j, carry):
            interleave(mm(2 * j, vbuf, ubuf), gen(2 * j + 1, vbuf2, ubuf2))
            interleave(mm(2 * j + 1, vbuf2, ubuf2), gen(jnp.minimum(2 * j + 2, NCH - 1), vbuf, ubuf))
            return carry

        jax.lax.fori_loop(0, NCH // 2, two, 0, unroll=2)

        fk_copy.wait()
        seen = set()
        lane_k = jax.lax.broadcasted_iota(jnp.int32, (D, 128), 1)
        for idx, (p, s0, s1, roll) in enumerate(pairs):
            ks = ps[pl.ds(s0, D, stride=16), :]
            if s1 >= 0:
                take = (lane_k % 64 >= 32) if roll == 32 else (lane_k == 1)
                ks = jnp.where(take, pltpu.roll(ps[pl.ds(s1, D, stride=16), :], roll, 1), ks)
            ks = ks.astype(bf)
            contrib = jax.lax.dot_general(fk_ref[idx], ks, (((1,), (1,)), ((), ())),
                                          preferred_element_type=f32)
            if p in seen:
                ksv[p] += contrib
            else:
                ksv[p] = contrib
                seen.add(p)
        H = BLK // 2
        for q in range(NB):
            for cc in range(4):
                for half, sg in ((0, 1.0), (1, -1.0)):
                    off = half * H + cc * (H // 4)
                    rr = pl.ds(off, H // 4)
                    ri = pl.ds(BLK + off, H // 4)
                    nr = sg * ksv[q, ri, :]
                    ni = -sg * ksv[q, rr, :]
                    if q > 0:
                        nr = nr + ksv[q - 1, rr, :]
                        ni = ni + ksv[q - 1, ri, :]
                    kf[q, rr, :] = nr
                    if q in S4:
                        kf[q, ri, :] = ni
                    else:
                        kf[q, ri, :] = nr + ni
                        kf[q, pl.ds(2 * BLK + off, H // 4), :] = ni - nr
        for c in copies():
            c.wait()

    z, b, xn = front(i)

    RC = 8
    src = [jnp.maximum(i - p, -1) + 1 for p in range(NB)]

    def mac(cc):
        t1 = t2 = t3 = t4 = None
        for p in range(NB):
            zr = zs[src[p], pl.ds(cc * RC, RC), :]
            zi = zs[src[p], pl.ds(BLK + cc * RC, RC), :]
            if p in S4:
                kr = kf[p, pl.ds(cc * RC, RC), :]
                ki = kf[p, pl.ds(BLK + cc * RC, RC), :]
                m2 = zi * ki
                m3 = zr * ki + zi * kr
                m4 = zr * kr
                t2 = m2 if t2 is None else t2 + m2
                t3 = m3 if t3 is None else t3 + m3
                t4 = m4 if t4 is None else t4 + m4
                continue
            zsum = zs[src[p], pl.ds(2 * BLK + cc * RC, RC), :]
            m1 = zsum * kf[p, pl.ds(cc * RC, RC), :]
            m2 = zi * kf[p, pl.ds(BLK + cc * RC, RC), :]
            m3 = zr * kf[p, pl.ds(2 * BLK + cc * RC, RC), :]
            t1 = m1 if t1 is None else t1 + m1
            t2 = m2 if t2 is None else t2 + m2
            t3 = m3 if t3 is None else t3 + m3
        yr = t1 - t2
        if t4 is not None:
            yr = yr + t4
        yi = t1 + t3
        hbuf[pl.ds(cc * RC, RC), :] = yr.astype(bf)
        hbuf[pl.ds(BLK + cc * RC, RC), :] = yi.astype(bf)

    nmac = 0
    late = []
    bounds = list(range(0, FF, FC)) + [FF]
    for k, (lo, hi) in enumerate(zip(bounds[:-1], bounds[1:])):
        a = jax.lax.dot_general(z, w3[lo:hi, :], (((1,), (1,)), ((), ())), preferred_element_type=f32)
        if k in PINS:
            zs[NB + 1, 0:BLK, 0:hi - lo] = a
            for _ in range(PINS[k]):
                mac(nmac)
                nmac += 1
            a = zs[NB + 1, 0:BLK, 0:hi - lo]
        h2 = jax.nn.gelu(a, approximate=True).astype(bf)
        if k in PINS:
            late.append((h2, lo, hi))
        else:
            b = b + jnp.dot(h2, w4[lo:hi, :], preferred_element_type=f32)
    assert nmac == BLK // RC
    for h2, lo, hi in late:
        b = b + jnp.dot(h2, w4[lo:hi, :], preferred_element_type=f32)

    y = jnp.dot(g_ref[...], hbuf[...], preferred_element_type=f32)
    s = y.astype(bf).astype(f32) + xn.astype(f32) * dsk_ref[...].astype(f32).reshape(1, D)
    g = b * jax.nn.sigmoid(b)
    xc = pl.ds(pl.multiple_of(i * BLK + HALO, HALO), BLK)
    o_ref[...] = (xs[xc, :].astype(f32) + s * g).astype(o_ref.dtype)


@jax.jit
def pallas_recurrent_scan__ssm_conv_s4__mixer_s_mlp__prompt_kernel(
    A_u, A_A_re, A_A_im, A_B_re, A_B_im, A_C_re, A_C_im, A_log_dt, A_Dskip,
    B_x, B_w1, B_w2, B_w3, B_w4,
):
    f, g, fk_all, pairs = _tables()
    bf = jnp.bfloat16
    f32 = jnp.float32
    x = A_u.reshape(L, D)
    ldt = A_log_dt
    dsk = A_Dskip

    def full(shape):
        return pl.BlockSpec(shape, lambda i: (0,) * len(shape))

    hbm = pl.BlockSpec(memory_space=pltpu.HBM)
    in_specs = [hbm] * 16
    scratch = [
        pltpu.VMEM((L + 2 * HALO, D), bf),
        pltpu.VMEM((D, D), bf), pltpu.VMEM((D, D), bf),
        pltpu.VMEM((FFP, D), bf), pltpu.VMEM((FFP, D), bf),
        pltpu.VMEM(f.shape, bf), pltpu.VMEM(g.shape, bf), pltpu.VMEM(fk_all.shape, bf),
        pltpu.SemaphoreType.DMA((8,)),
    ] + [pltpu.VMEM((D, N), bf)] * 6 + [pltpu.VMEM((D,), bf), pltpu.VMEM((D,), bf),
        pltpu.SemaphoreType.DMA((8,)),
        pltpu.VMEM((D, N), f32), pltpu.VMEM((D, N), f32),
        pltpu.VMEM((D, N), f32), pltpu.VMEM((D, N), f32),
        pltpu.VMEM((128 * CH, N), f32),
        pltpu.VMEM((64 * CH, N), f32),
        pltpu.VMEM((128 * CH, N), f32), pltpu.VMEM((64 * CH, N), f32),
        pltpu.VMEM((D * 16, 128), f32),
        pltpu.VMEM((NB, 3 * BLK, D), f32),
        pltpu.VMEM((NB, 2 * BLK, D), f32),
        pltpu.VMEM((NB + 2, 3 * BLK, D), f32),
        pltpu.VMEM((2 * BLK, D), bf),
    ]
    out = pl.pallas_call(
        functools.partial(_kernel, pairs),
        grid=(NB,),
        in_specs=in_specs,
        out_specs=pl.BlockSpec((BLK, D), lambda i: (i, 0)),
        out_shape=jax.ShapeDtypeStruct((L, D), bf),
        scratch_shapes=scratch,
        compiler_params=pltpu.CompilerParams(
            dimension_semantics=("arbitrary",),
            vmem_limit_bytes=128 * 1024 * 1024),
    )(x, A_A_re, A_A_im, A_B_re, A_B_im, A_C_re, A_C_im, ldt, dsk,
      B_w1, B_w2, B_w3.T, B_w4,
      jnp.asarray(f, bf), jnp.asarray(g, bf), jnp.asarray(fk_all, bf))
    return out.reshape(1, L, D)
```
